```python
import os as _os
_os.environ.setdefault("JAX_PLATFORMS", "cpu")
import jax
import jax.numpy as jnp

def _softmax(x, axis=-1):
    return jax.nn.softmax(x, axis=axis)
def _gelu(x):
    return jax.nn.gelu(x, approximate=True)
def _silu(x):
    return jax.nn.silu(x)
def _sigmoid(x):
    return jax.nn.sigmoid(x)
def _layernorm(x, axis=-1, eps=1e-5):
    m = jnp.mean(x, axis=axis, keepdims=True)
    v = jnp.var(x, axis=axis, keepdims=True)
    return (x - m) / jnp.sqrt(v + eps)
def _scatter_add(tgt, idx, src, axis=0):
    return tgt.at[idx].add(src)
def _segment_sum(src, seg, n):
    return jax.ops.segment_sum(src, seg, n)
class _Rng:
    def __init__(self, key):
        self._k = key
    def _next(self):
        self._k, sub = jax.random.split(self._k)
        return sub
    def normal(self, shape):
        return jax.random.normal(self._next(), shape, dtype=jnp.bfloat16)
    def randint(self, lo, hi, shape):
        return jax.random.randint(self._next(), shape, lo, hi, dtype=jnp.int32)
    def uniform(self, shape, lo=0.0, hi=1.0):
        return jax.random.uniform(self._next(), shape, jnp.bfloat16, lo, hi)
    def permutation(self, n):
        return jax.random.permutation(self._next(), n)


kernel_name = 'gated_mix__sliding_block__sliding_local_dilated__prompt'

def setup_inputs():
    _rng = _Rng(jax.random.key(int.from_bytes(__import__("os").urandom(4), "little")))
    _w = (lambda a: (lambda t: t.astype(jnp.bfloat16) if jnp.issubdtype(t.dtype, jnp.floating) else t)(jnp.asarray(a)))
    def _A_setup():
        B, S, D = 1, 2048, 640
        return {
            "x": _w((lambda *s: _rng.normal(s) * 0.05)(B, S, D)),
            "wqkv": _w((lambda *s: _rng.normal(s) * 0.8)(D, 3 * D)),
            "wo": _w((lambda *s: _rng.normal(s) * 0.05)(D, D)),
        }
    _A_in = _A_setup()

    def _B_setup():
        B, S, D = 1, 2048, 640
        return {
            "x": _w((lambda *s: _rng.normal(s) * 0.05)(B, S, D)),
            "wqkv": _w((lambda *s: _rng.normal(s) * 0.8)(D, 3 * D)),
            "wo": _w((lambda *s: _rng.normal(s) * 0.05)(D, D)),
        }
    _B_in = _B_setup()

    return {
        "A_x": _A_in["x"],
        "A_wqkv": _A_in["wqkv"],
        "A_wo": _A_in["wo"],
        "B_x": _B_in["x"],
        "B_wqkv": _B_in["wqkv"],
        "B_wo": _B_in["wo"],
        "gate_w": _w((lambda *s: _rng.normal(s) * 0.05)(640) * 16.0),
    }

def reference(A_x, A_wqkv, A_wo, B_x, B_wqkv, B_wo, gate_w):
    def _A_ref(x, wqkv, wo):
        B, S, D = x.shape
        H = 32; Dh = D // H; W = 256
        qkv = (lambda x, *d: x.transpose(*d))((x @ wqkv).reshape(B, S, 3, H, Dh), 2, 0, 3, 1, 4)
        q, k, v = qkv[0], qkv[1], qkv[2]
        scores = jnp.einsum("bhqd,bhkd->bhqk", q, k) * (Dh ** -0.5)
        idx = jnp.arange(S)
        mask = (idx[:, None] - idx[None, :] >= 0) & (idx[:, None] - idx[None, :] < W)
        scores = jnp.where(mask[None, None], scores, -1e9)
        p = _softmax(scores, axis=-1)
        o = jnp.einsum("bhqk,bhkd->bhqd", p, v)
        return (lambda x, *d: x.transpose(*d))(o, 0, 2, 1, 3).reshape(B, S, D) @ wo

    def _B_ref(x, wqkv, wo):
        B, S, D = x.shape
        H = 32; Dh = D // H
        W, dil = 8, 2
        qkv = (lambda x, *d: x.transpose(*d))((x @ wqkv).reshape(B, S, 3, H, Dh), 2, 0, 3, 1, 4)
        q, k, v = qkv[0], qkv[1], qkv[2]
        scale = Dh ** -0.5
        pos = jnp.arange(S)
        off = jnp.arange(W) * dil
        idx = pos[:, None] - off[None, :]
        mask = idx >= 0
        idx_c = jnp.where(mask, idx, 0).reshape(-1)
        kg = k[:, :, idx_c, :].reshape(B, H, S, W, Dh)
        vg = v[:, :, idx_c, :].reshape(B, H, S, W, Dh)
        logits = jnp.einsum("bhsd,bhswd->bhsw", q, kg) * scale
        logits = jnp.where(mask[None, None, :, :], logits, -1e9)
        attn = _softmax(logits, axis=-1)
        o = jnp.einsum("bhsw,bhswd->bhsd", attn, vg)
        return (lambda x, *d: x.transpose(*d))(o, 0, 2, 1, 3).reshape(B, S, D) @ wo

    x = A_x
    g = _sigmoid((x * gate_w).sum(-1, keepdims=True))
    a = _A_ref(x, A_wqkv, A_wo)
    b = _B_ref(x, B_wqkv, B_wo)
    return g * a + (1 - g) * b
```

```python
import functools
import numpy as np
import jax
import jax.numpy as jnp
from jax import lax
import jax.experimental.pallas as pl
import jax.experimental.pallas.tpu as pltpu

S, D, H, DH = 2048, 640, 32, 20
BQ = 128
NB = S // BQ
NT = D // 128
HD = D // 2
NEG = -1e30
LOG2E = 1.4426950408889634
QS = (DH ** -0.5) * LOG2E
F32, BF16, U32 = jnp.float32, jnp.bfloat16, jnp.uint32
AHEAD = 1


def _iota(shape, dim):
    return lax.broadcasted_iota(jnp.int32, shape, dim)


def _dot(a, b):
    return jnp.dot(a, b, preferred_element_type=F32)


def _dot_nt(a, b):
    return lax.dot_general(a, b, (((1,), (1,)), ((), ())), preferred_element_type=F32)


def _pk(x):
    return pltpu.bitcast(x.astype(BF16), U32)


def _up(x):
    return pltpu.bitcast(x, BF16)


class R:
    pass


def _proj_pieces(r, j, p, xa_ref):
    def lanes(t):
        return slice(t * 128, (t + 1) * 128)

    def qa(t):
        q = _dot(xa_ref[...], _up(r.wa[:, t * 128:(t + 1) * 128])) * QS
        r.qT[p, t * 64:(t + 1) * 64, :] = pltpu.bitcast(q.astype(BF16).T, U32)

    def ka(t):
        k = _pk(_dot(xa_ref[...], _up(r.wa[:, D + t * 128:D + (t + 1) * 128])))
        r.ka[j + 2, t] = k
        r.kr[p, t] = pltpu.roll(k[32:64], 64, 1)

    def va(t):
        v = _dot(xa_ref[...], _up(r.wa[:, 2 * D + t * 128:2 * D + (t + 1) * 128]))
        r.va[j + 2, t * 64:(t + 1) * 64, :] = pltpu.bitcast(v.astype(BF16).T, U32)

    def qb(t):
        r.qb[p, t] = _dot_nt(xa_ref[...], _up(r.wbT[t * 64:(t + 1) * 64, :])) * QS

    def kb(t):
        r.kb[p, t, 16:16 + BQ, :] = _dot_nt(xa_ref[...], _up(r.wbT[HD + t * 64:HD + (t + 1) * 64, :]))

    def vb(t):
        r.vb[p, t, 16:16 + BQ, :] = _dot_nt(xa_ref[...], _up(r.wbT[2 * HD + t * 64:2 * HD + (t + 1) * 64, :]))

    def gate():
        z = jnp.sum(xa_ref[...].astype(F32) * r.gw[...].astype(F32), axis=-1, keepdims=True)
        r.g[p] = jnp.broadcast_to(1.0 / (1.0 + jnp.exp(-z)), (BQ, 128))

    out = [functools.partial(f, t) for f in (qa, ka, va, qb, kb, vb) for t in range(NT)]
    return out, gate


def _qk(r, h, i, p):
    f0 = DH * h
    t, off = divmod(f0, 128)
    straddle = off + DH > 128
    lane = _iota((8, 128), 1)

    def ktile(blk, r0, r1):
        a = r.ka[i + blk, t, r0:r1, :]
        if straddle:
            a = jnp.where(_iota((r1 - r0, 128), 1) >= off, a, r.ka[i + blk, t + 1, r0:r1, :])
        return a

    zero = jnp.zeros((8, 128), U32)
    sub = _iota((8, 128), 0)
    left = lane < 64
    qm, qc = [zero] * 8, [zero] * 8
    for v in range(8):
        rows = [(8 * v + s - off // 2) % 64 < DH // 2 for s in range(8)]
        if not any(rows):
            continue
        tt = t if (not straddle or 8 * v + 7 >= off // 2) else t + 1
        x = r.qT[p, tt * 64 + 8 * v: tt * 64 + 8 * v + 8, :]
        if not all(rows):
            lo = rows.index(True)
            hi = lo + sum(rows)
            x = jnp.where((sub >= lo) & (sub < hi), x, zero)
        qm[v] = x
        qc[v] = jnp.where(left, x, zero)
        qc[(v + 4) % 8] = jnp.where(left, zero, x)
    qh = _up(jnp.concatenate(qm, axis=0))
    qcor = _up(jnp.concatenate(qc, axis=0))
    l32 = _iota((32, 128), 1)
    lm = ((l32 - off) & 127) < DH
    kmain = jnp.concatenate([ktile(0, 32, 64), ktile(1, 0, 64), ktile(2, 0, 32)], axis=0)
    krot = r.kr[p, t]
    if straddle:
        krot = jnp.where(((l32 - 64) & 127) >= off, krot, r.kr[p, t + 1])
    kcor = jnp.where(lm, ktile(0, 0, 32), krot)
    return _dot(_up(kmain), qh), _dot(_up(kcor), qcor)


def _softmax(r, s_main, s_cor, c):
    rows = []
    for v in range(8):
        cond = c.dsub <= -8 * v
        rows.append(jnp.where(cond, s_main[192 + 8 * v:200 + 8 * v],
                              jnp.where(c.valid0, s_cor[8 * v:8 * v + 8], NEG)))
    for v in range(8):
        cond = c.dsub <= -8 * (v + 8)
        rows.append(jnp.where(cond, s_cor[8 * v:8 * v + 8],
                              jnp.where(c.valid0, s_main[8 * v:8 * v + 8], NEG)))
    sm = jnp.concatenate(rows, axis=0)
    s1 = s_main[64:192]
    mx = jnp.maximum(jnp.max(sm, axis=0, keepdims=True),
                     jnp.max(s1, axis=0, keepdims=True) - c.big1)
    pm = jnp.exp2(sm - mx)
    p1 = jnp.exp2(s1 - (mx + c.big1))
    l = jnp.sum(pm + p1, axis=0, keepdims=True)
    pmb = _pk(pm)
    dm = r.pm[...]
    pall = jnp.concatenate([_up(pmb & ~dm), p1.astype(BF16), _up(pmb & dm)], axis=0)
    return pall, l


def _pv(r, h, i, pall, l):
    f0 = DH * h
    rb = (f0 // 16) * 8
    ro = f0 % 16
    vT = jnp.concatenate([r.va[i + b, rb:rb + 16, :] for b in range(3)], axis=1)
    o = _dot(_up(vT), pall) * (1.0 / l)
    r.oT[f0:f0 + DH, :] = o[ro:ro + DH, :]


def _attn_b(r, i, p, g):
    pos = i * BQ + g * 8 + _iota((8, 128), 0)
    r0 = 16 + 8 * g
    lg = []
    for w in range(8):
        acc = None
        for t in range(NT):
            x = r.qb[p, t, 8 * g:8 * g + 8, :] * r.kb[p, t, r0 - 2 * w:r0 - 2 * w + 8, :]
            acc = x if acc is None else acc + x
        acc = acc + pltpu.roll(acc, 64, 1)
        acc = acc + pltpu.roll(acc, 32, 1)
        if w > 0 and g < 2:
            acc = jnp.where(pos >= 2 * w, acc, NEG)
        lg.append(acc)
    mxb = functools.reduce(jnp.maximum, lg)
    pb = [jnp.exp2(x - mxb) for x in lg]
    inv = 1.0 / functools.reduce(lambda x, y: x + y, pb)
    for t in range(NT):
        acc = None
        for w in range(8):
            x = pb[w] * r.vb[p, t, r0 - 2 * w:r0 - 2 * w + 8, :]
            acc = x if acc is None else acc + x
        r.ob[8 * g:8 * g + 8, t * 128:(t + 1) * 128] = acc * inv


def _kernel(xa0_ref, xa_ref, wa_ref, woa_ref, wb_ref, wob_ref, gw_ref, o_ref,
            wa_s, wbT_s, wo_s, tmp_s, pm_s, qT_s, ka_s, kr_s, va_s, qb_s, kb_s, vb_s, g_s, oT_s, ob_s):
    i = pl.program_id(0)
    r = R()
    r.gw, r.wa, r.wbT, r.wo, r.pm, r.qT, r.ka, r.kr, r.va = gw_ref, wa_s, wbT_s, wo_s, pm_s, qT_s, ka_s, kr_s, va_s
    r.qb, r.kb, r.vb, r.g, r.oT, r.ob = qb_s, kb_s, vb_s, g_s, oT_s, ob_s

    @pl.when(i == 0)
    def _prologue():
        wa_s[...] = pltpu.bitcast(wa_ref[...], U32)
        wo_s[0:HD, :] = pltpu.bitcast(woa_ref[...], U32)
        for m in range(3):
            wt = wb_ref[:, m * D:(m + 1) * D].astype(F32).T
            for t in range(NT):
                tmp_s[t] = wt[:, t * 128:(t + 1) * 128]
            for t in range(NT):
                for d in range(DH):
                    wbT_s[pl.ds(m * HD + d * 16, 16), t * 128:(t + 1) * 128] = _pk(tmp_s[t, pl.ds(d, 32, stride=DH), :])
        wt = wob_ref[...].astype(F32)
        for t in range(NT):
            tmp_s[t] = wt[:, t * 128:(t + 1) * 128]
        for t in range(NT):
            for d in range(DH):
                wo_s[pl.ds(HD + d * 16, 16), t * 128:(t + 1) * 128] = _pk(tmp_s[t, pl.ds(d, 32, stride=DH), :])
        ka_s[0:2] = jnp.zeros((2, NT, 64, 128), U32)
        va_s[0:2] = jnp.zeros((2, HD, BQ), U32)
        kb_s[0, :, 0:16, :] = jnp.zeros((NT, 16, 128), F32)
        vb_s[0, :, 0:16, :] = jnp.zeros((NT, 16, 128), F32)
        rr = 2 * _iota((64, 128), 0)
        cc = _iota((64, 128), 1)
        pm_s[...] = (jnp.where(rr <= cc, jnp.uint32(0xFFFF), jnp.uint32(0))
                     | jnp.where(rr + 1 <= cc, jnp.uint32(0xFFFF0000), jnp.uint32(0)))
        pieces, gate = _proj_pieces(r, 0, 0, xa0_ref)
        for f in pieces:
            f()
        gate()

    def body(p, do_proj):
        c = R()
        c.dsub = _iota((8, 128), 0) - _iota((8, 128), 1)
        c.valid0 = i >= 2
        c.big1 = jnp.where(i >= 1, 0.0, 1e30).astype(F32)
        pieces = []
        if do_proj:
            kb_s[1 - p, :, 0:16, :] = kb_s[p, :, BQ:BQ + 16, :]
            vb_s[1 - p, :, 0:16, :] = vb_s[p, :, BQ:BQ + 16, :]
            pieces, gate = _proj_pieces(r, i + 1, 1 - p, xa_ref)
            gate()
        sq = {}
        for h in range(min(AHEAD, H)):
            sq[h] = _qk(r, h, i, p)
        for h in range(H):
            if h + AHEAD < H:
                sq[h + AHEAD] = _qk(r, h + AHEAD, i, p)
            pall, l = _softmax(r, *sq.pop(h), c)
            if h < len(pieces):
                pieces[h]()
            _pv(r, h, i, pall, l)
            if h % 2 == 0:
                _attn_b(r, i, p, h // 2)
        b = _dot(ob_s[...].astype(BF16), _up(wo_s[HD:D, :]))
        oa = oT_s[...].astype(BF16).T
        a = _dot(oa, _up(wo_s[0:HD, :]))
        g = g_s[p]
        g5 = jnp.concatenate([g] * NT, axis=1)
        o_ref[...] = (b + g5 * (a - b)).astype(o_ref.dtype)

    for p in range(2):
        @pl.when((i % 2 == p) & (i < NB - 1))
        def _():
            body(p, True)

    @pl.when(i == NB - 1)
    def _():
        body((NB - 1) % 2, False)


@jax.jit
def pallas_gated_mix__sliding_block__sliding_local_dilated__prompt_kernel(A_x, A_wqkv, A_wo, B_x, B_wqkv, B_wo, gate_w):
    full = lambda shp: pl.BlockSpec(shp, lambda i: (0,) * len(shp))
    x0 = pl.BlockSpec((BQ, D), lambda i: (0, 0))
    xn = pl.BlockSpec((BQ, D), lambda i: (jnp.minimum(i + 1, NB - 1), 0))
    xs = pl.BlockSpec((BQ, D), lambda i: (i, 0))
    xa = A_x.reshape(S, D)
    out = pl.pallas_call(
        _kernel,
        grid=(NB,),
        in_specs=[x0, xn, full((D, 3 * D)), full((D, D)), full((D, 3 * D)), full((D, D)), full((1, D))],
        out_specs=xs,
        out_shape=jax.ShapeDtypeStruct((S, D), BF16),
        scratch_shapes=[
            pltpu.VMEM((HD, 3 * D), U32), pltpu.VMEM((3 * HD, D), U32), pltpu.VMEM((D, D), U32),
            pltpu.VMEM((NT, D, 128), F32), pltpu.VMEM((64, 128), U32),
            pltpu.VMEM((2, HD, BQ), U32),
            pltpu.VMEM((NB + 2, NT, 64, 128), U32), pltpu.VMEM((2, NT, 32, 128), U32),
            pltpu.VMEM((NB + 2, HD, BQ), U32),
            pltpu.VMEM((2, NT, BQ, 128), F32),
            pltpu.VMEM((2, NT, BQ + 16, 128), F32), pltpu.VMEM((2, NT, BQ + 16, 128), F32),
            pltpu.VMEM((2, BQ, 128), F32),
            pltpu.VMEM((D, BQ), F32), pltpu.VMEM((BQ, D), F32),
        ],
        compiler_params=pltpu.CompilerParams(dimension_semantics=("arbitrary",),
                                             vmem_limit_bytes=100 * 1024 * 1024),
        name="gmix",
    )(xa, xa, A_wqkv, A_wo, B_wqkv, B_wo, gate_w.reshape(1, D))
    return out.reshape(1, S, D)
```

```python
import functools
import numpy as np
import jax
import jax.numpy as jnp
from jax import lax
import jax.experimental.pallas as pl
import jax.experimental.pallas.tpu as pltpu

S, D, H, DH = 2048, 640, 32, 20
BQ = 128
NB = S // BQ
NT = D // 128
HD = D // 2
NEG = -1e30
LOG2E = 1.4426950408889634
QS = (DH ** -0.5) * LOG2E
F32, BF16, U32 = jnp.float32, jnp.bfloat16, jnp.uint32
AHEAD = 3
PLACE=0
ORD=0
BST=0
NS = NB // 2


def _iota(shape, dim):
    return lax.broadcasted_iota(jnp.int32, shape, dim)


def _dot(a, b):
    return jnp.dot(a, b, preferred_element_type=F32)


def _dot_nt(a, b):
    return lax.dot_general(a, b, (((1,), (1,)), ((), ())), preferred_element_type=F32)


def _pk(x):
    return pltpu.bitcast(x.astype(BF16), U32)


def _up(x):
    return pltpu.bitcast(x, BF16)


class R:
    pass


def _proj_pieces(r, j, p):
    xs = r.x.at[pl.ds(pl.multiple_of(j * BQ, BQ), BQ), :] if not isinstance(j, int) else r.x.at[pl.ds(j * BQ, BQ), :]
    def lanes(t):
        return slice(t * 128, (t + 1) * 128)

    def qa(t):
        q = _dot(xs[...], _up(r.wa[:, t * 128:(t + 1) * 128])) * QS
        r.qT[p, t * 64:(t + 1) * 64, :] = pltpu.bitcast(q.astype(BF16).T, U32)

    def ka(t):
        k = _pk(_dot(xs[...], _up(r.wa[:, D + t * 128:D + (t + 1) * 128])))
        r.ka[j + 2, t] = k
        r.kr[p, t] = pltpu.roll(k[32:64], 64, 1)

    def va(t):
        v = _dot(xs[...], _up(r.wa[:, 2 * D + t * 128:2 * D + (t + 1) * 128]))
        r.va[j + 2, t * 64:(t + 1) * 64, :] = pltpu.bitcast(v.astype(BF16).T, U32)

    def qb(t):
        r.qb[p, t] = _dot_nt(xs[...], _up(r.wbT[t * 64:(t + 1) * 64, :])) * QS

    def kb(t):
        r.kb[p, t, 16:16 + BQ, :] = _dot_nt(xs[...], _up(r.wbT[HD + t * 64:HD + (t + 1) * 64, :]))

    def vb(t):
        r.vb[p, t, 16:16 + BQ, :] = _dot_nt(xs[...], _up(r.wbT[2 * HD + t * 64:2 * HD + (t + 1) * 64, :]))

    def gate():
        z = jnp.sum(xs[...].astype(F32) * r.gw[...].astype(F32).reshape(1, D), axis=-1, keepdims=True)
        r.g[j + 2] = jnp.broadcast_to(1.0 / (1.0 + jnp.exp(-z)), (BQ, 128))

    out = [functools.partial(f, t) for f in (qa, ka, va, qb, kb, vb) for t in range(NT)]
    if ORD == 1 and not isinstance(j, int):
        out = [functools.partial(f, t) for f in (qb, kb, vb, qa, ka, va) for t in range(NT)]
    if ORD == 2 and not isinstance(j, int):
        out = [functools.partial(f, t) for t in range(NT) for f in (qa, ka, va, qb, kb, vb)]
    return out, gate


def _qk(r, h, i, p):
    f0 = DH * h
    t, off = divmod(f0, 128)
    straddle = off + DH > 128
    lane = _iota((8, 128), 1)

    def ktile(blk, r0, r1):
        a = r.ka[i + blk, t, r0:r1, :]
        if straddle:
            a = jnp.where(_iota((r1 - r0, 128), 1) >= off, a, r.ka[i + blk, t + 1, r0:r1, :])
        return a

    zero = jnp.zeros((8, 128), U32)
    sub = _iota((8, 128), 0)
    left = lane < 64
    qm, qc = [zero] * 8, [zero] * 8
    for v in range(8):
        rows = [(8 * v + s - off // 2) % 64 < DH // 2 for s in range(8)]
        if not any(rows):
            continue
        tt = t if (not straddle or 8 * v + 7 >= off // 2) else t + 1
        x = r.qT[p, tt * 64 + 8 * v: tt * 64 + 8 * v + 8, :]
        if not all(rows):
            lo = rows.index(True)
            hi = lo + sum(rows)
            x = jnp.where((sub >= lo) & (sub < hi), x, zero)
        qm[v] = x
        qc[v] = jnp.where(left, x, zero)
        qc[(v + 4) % 8] = jnp.where(left, zero, x)
    qh = _up(jnp.concatenate(qm, axis=0))
    qcor = _up(jnp.concatenate(qc, axis=0))
    l32 = _iota((32, 128), 1)
    lm = ((l32 - off) & 127) < DH
    kmain = jnp.concatenate([ktile(0, 32, 64), ktile(1, 0, 64), ktile(2, 0, 32)], axis=0)
    krot = r.kr[p, t]
    if straddle:
        krot = jnp.where(((l32 - 64) & 127) >= off, krot, r.kr[p, t + 1])
    kcor = jnp.where(lm, ktile(0, 0, 32), krot)
    if True:
        n=2; sm = jnp.concatenate([_dot(_up(kmain[k*128//n:(k+1)*128//n]), qh) for k in range(n)], axis=0)
        return sm, _dot(_up(kcor), qcor)
    return _dot(_up(kmain), qh), _dot(_up(kcor), qcor)


def _softmax(r, s_main, s_cor, c):
    rows = []
    for v in range(8):
        cond = c.dsub <= -8 * v
        rows.append(jnp.where(cond, s_main[192 + 8 * v:200 + 8 * v],
                              jnp.where(c.valid0, s_cor[8 * v:8 * v + 8], NEG)))
    for v in range(8):
        cond = c.dsub <= -8 * (v + 8)
        rows.append(jnp.where(cond, s_cor[8 * v:8 * v + 8],
                              jnp.where(c.valid0, s_main[8 * v:8 * v + 8], NEG)))
    sm = jnp.concatenate(rows, axis=0)
    s1 = s_main[64:192]
    mx = jnp.maximum(jnp.max(sm, axis=0, keepdims=True),
                     jnp.max(s1, axis=0, keepdims=True) - c.big1)
    pm = jnp.exp2(sm - mx)
    p1 = jnp.exp2(s1 - (mx + c.big1))
    l = jnp.sum(pm + p1, axis=0, keepdims=True)
    pmb = _pk(pm)
    dm = r.pm[...]
    pall = jnp.concatenate([_up(pmb & ~dm), p1.astype(BF16), _up(pmb & dm)], axis=0)
    return pall, l


def _pv(r, h, i, p, pall, l):
    f0 = DH * h
    rb = (f0 // 16) * 8
    ro = f0 % 16
    vT = jnp.concatenate([r.va[i + b, rb:rb + 16, :] for b in range(3)], axis=1)
    o = _dot(_up(vT), pall) * (1.0 / l)
    r.oT[p, f0:f0 + DH, :] = o[ro:ro + DH, :]


def _attn_b(r, i, p, g):
    pos = i * BQ + g * 8 + _iota((8, 128), 0)
    r0 = 16 + 8 * g
    lg = []
    for w in range(8):
        acc = None
        for t in range(NT):
            x = r.qb[p, t, 8 * g:8 * g + 8, :] * r.kb[p, t, r0 - 2 * w:r0 - 2 * w + 8, :]
            acc = x if acc is None else acc + x
        acc = acc + pltpu.roll(acc, 64, 1)
        acc = acc + pltpu.roll(acc, 32, 1)
        if w > 0 and g < 2:
            acc = jnp.where(pos >= 2 * w, acc, NEG)
        lg.append(acc)
    mxb = functools.reduce(jnp.maximum, lg)
    pb = [jnp.exp2(x - mxb) for x in lg]
    inv = 1.0 / functools.reduce(lambda x, y: x + y, pb)
    for t in range(NT):
        acc = None
        for w in range(8):
            x = pb[w] * r.vb[p, t, r0 - 2 * w:r0 - 2 * w + 8, :]
            acc = x if acc is None else acc + x
        r.ob[p, 8 * g:8 * g + 8, t * 128:(t + 1) * 128] = acc * inv


def _out_pieces(r, blk, p):
    def piece(t):
        cs = slice(t * 128, (t + 1) * 128)
        b = _dot(r.obb[...], _up(r.wo[HD:D, cs]))
        a = _dot(_up(r.oa[...]), _up(r.wo[0:HD, cs]))
        r.out[blk + 2, :, cs] = (b + r.g[blk + 2] * (a - b)).astype(BF16)

    def prep():
        r.oa[...] = pltpu.bitcast(r.oT[p].astype(BF16).T, U32)
        r.obb[...] = r.ob[p].astype(BF16)

    return prep, [functools.partial(piece, t) for t in range(NT)]


def _block(r, i, p, do_proj):
    c = R()
    c.dsub = _iota((8, 128), 0) - _iota((8, 128), 1)
    c.valid0 = i >= 2
    c.big1 = jnp.where(i >= 1, 0.0, 1e30).astype(F32)
    prep, opcs = _out_pieces(r, i - 2, p)
    prep()
    pieces = []
    if do_proj:
        r.kb[1 - p, :, 0:16, :] = r.kb[p, :, BQ:BQ + 16, :]
        r.vb[1 - p, :, 0:16, :] = r.vb[p, :, BQ:BQ + 16, :]
        ppcs, gate = _proj_pieces(r, i + 1, 1 - p)
    else:
        ppcs, gate = [], None
    n = len(ppcs) + 2 * len(opcs)
    order = []
    oi = 0
    for k, f in enumerate(ppcs):
        order.append(f)
        if k % 6 == 3:
            order.append(opcs[oi]); oi += 1
    order += opcs[oi:]
    if gate is not None and False:
        gate()
    sq = {}
    for h in range(AHEAD):
        sq[h] = _qk(r, h, i, p)
    done = 0
    for h in range(H):
        if h + AHEAD < H:
            sq[h + AHEAD] = _qk(r, h + AHEAD, i, p)
        if PLACE == 0:
            pall, l = _softmax(r, *sq.pop(h), c)
        want = ((h + 1) * len(order) + H - 1) // H if do_proj else min(len(order), (h + 1) // 4)
        while done < min(want, len(order)):
            order[done](); done += 1
        if PLACE == 1:
            pall, l = _softmax(r, *sq.pop(h), c)
        _pv(r, h, i, p, pall, l)
        if BST < 2:
            if h % 2 == BST:
                _attn_b(r, i, p, h // 2)
        elif BST == 2:
            if h < 16:
                _attn_b(r, i, p, h)
        elif BST == 3:
            if 4 <= h < 28 and (h - 4) % 3 != 2:
                _attn_b(r, i, p, (h - 4) - (h - 4) // 3)
    while done < len(order):
        order[done](); done += 1
    if gate is not None and True:
        gate()


def _kernel(x_hbm, wa_hbm, woa_hbm, wb_hbm, wob_hbm, gw_ref, o_hbm,
            x_s, wraw_s, woraw_s, wa_s, wbT_s, wo_s, tmp_s, pm_s, qT_s, ka_s, kr_s, va_s,
            qb_s, kb_s, vb_s, g_s, oT_s, ob_s, oa_s, obb_s, out_s, sem, xsem, osem):
    s = pl.program_id(0)
    r = R()
    r.x, r.gw, r.wa, r.wbT, r.wo, r.pm, r.qT, r.ka, r.kr, r.va = x_s, gw_ref, wa_s, wbT_s, wo_s, pm_s, qT_s, ka_s, kr_s, va_s
    r.qb, r.kb, r.vb, r.g, r.oT, r.ob, r.oa, r.obb, r.out = qb_s, kb_s, vb_s, g_s, oT_s, ob_s, oa_s, obb_s, out_s

    def out_copy(b):
        return pltpu.make_async_copy(out_s.at[b + 2], o_hbm.at[pl.ds(b * BQ, BQ), :], osem)

    def wcopy(c):
        src, slot = (wb_hbm, 1) if c % 2 == 0 else (wa_hbm, 0)
        cs = pl.ds((c // 2) * D, D)
        return pltpu.make_async_copy(src.at[:, cs], wraw_s.at[slot, :, cs], sem.at[c])

    def ocopy(k):
        return pltpu.make_async_copy((woa_hbm, wob_hbm)[k], woraw_s.at[k], sem.at[7 + k])

    def xcopy(k):
        if not isinstance(k, int):
            raise NotImplementedError
        n = 2 * BQ if k < NS - 1 else BQ
        return pltpu.make_async_copy(x_hbm.at[pl.ds((2 * k + 1) * BQ, n), :],
                                     x_s.at[pl.ds((2 * k + 1) * BQ, n), :], xsem.at[k])

    @pl.when(s == 0)
    def _prologue():
        cx0 = pltpu.make_async_copy(x_hbm.at[pl.ds(0, BQ), :], x_s.at[pl.ds(0, BQ), :], sem.at[6])
        cx0.start()
        wcopy(0).start(); wcopy(1).start()
        ka_s[0:2] = jnp.zeros((2, NT, 64, 128), U32)
        va_s[0:2] = jnp.zeros((2, HD, BQ), U32)
        kb_s[0, :, 0:16, :] = jnp.zeros((NT, 16, 128), F32)
        vb_s[0, :, 0:16, :] = jnp.zeros((NT, 16, 128), F32)
        rr = 2 * _iota((64, 128), 0)
        cc = _iota((64, 128), 1)
        pm_s[...] = (jnp.where(rr <= cc, jnp.uint32(0xFFFF), jnp.uint32(0))
                     | jnp.where(rr + 1 <= cc, jnp.uint32(0xFFFF0000), jnp.uint32(0)))
        pieces, gate = _proj_pieces(r, 0, 0)
        cx0.wait()
        for c in range(6):
            wcopy(c).wait()
            if c + 2 < 6:
                wcopy(c + 2).start()
            elif c == 4:
                xcopy(0).start()
            else:
                ocopy(0).start(); ocopy(1).start()
                for k in range(1, NS):
                    xcopy(k).start()
            m = c // 2
            if c % 2 == 0:
                wt = wraw_s[1, :, m * D:(m + 1) * D].astype(F32).T
                for t in range(NT):
                    tmp_s[t] = wt[:, t * 128:(t + 1) * 128]
                for t in range(NT):
                    for d in range(DH):
                        wbT_s[pl.ds(m * HD + d * 16, 16), t * 128:(t + 1) * 128] = _pk(tmp_s[t, pl.ds(d, 32, stride=DH), :])
                todo = pieces[10 + 5 * m:15 + 5 * m] if m > 0 else []
            else:
                wa_s[:, m * D:(m + 1) * D] = pltpu.bitcast(wraw_s[0, :, m * D:(m + 1) * D], U32)
                todo = pieces[5 * m:5 * m + 5]
            for f in todo:
                f()
        for f in pieces[25:]:
            f()
        gate()

    @pl.when(s == 1)
    def _():
        ocopy(0).wait(); ocopy(1).wait()
        wo_s[0:HD, :] = pltpu.bitcast(woraw_s[0], U32)
        wt = woraw_s[1].astype(F32)
        for t in range(NT):
            tmp_s[t] = wt[:, t * 128:(t + 1) * 128]
        for t in range(NT):
            for d in range(DH):
                wo_s[pl.ds(HD + d * 16, 16), t * 128:(t + 1) * 128] = _pk(tmp_s[t, pl.ds(d, 32, stride=DH), :])

    for k in range(NS):
        @pl.when(s == k)
        def _():
            xcopy(k).wait()

    @pl.when(s < NS - 1)
    def _():
        _block(r, 2 * s, 0, True)
        _block(r, 2 * s + 1, 1, True)

    @pl.when(s == NS - 1)
    def _():
        _block(r, NB - 2, 0, True)
        _block(r, NB - 1, 1, False)
        for blk in (NB - 2, NB - 1):
            prep, opcs = _out_pieces(r, blk, blk % 2)
            prep()
            for f in opcs:
                f()

    @pl.when(s > 0)
    def _():
        out_copy(2 * s - 2).start()
        out_copy(2 * s - 1).start()

    @pl.when(s == NS - 1)
    def _():
        out_copy(NB - 2).start()
        out_copy(NB - 1).start()
        for b in range(NB):
            out_copy(b).wait()


@jax.jit
def pallas_gated_mix__sliding_block__sliding_local_dilated__prompt_kernel(A_x, A_wqkv, A_wo, B_x, B_wqkv, B_wo, gate_w):
    del B_x
    anyspec = pl.BlockSpec(memory_space=pl.ANY)
    out = pl.pallas_call(
        _kernel,
        grid=(NS,),
        in_specs=[anyspec] * 5 + [pl.BlockSpec((D,), lambda i: (0,))],
        out_specs=anyspec,
        out_shape=jax.ShapeDtypeStruct((S, D), BF16),
        scratch_shapes=[
            pltpu.VMEM((S, D), BF16), pltpu.VMEM((2, D, 3 * D), BF16), pltpu.VMEM((2, D, D), BF16),
            pltpu.VMEM((HD, 3 * D), U32), pltpu.VMEM((3 * HD, D), U32), pltpu.VMEM((D, D), U32),
            pltpu.VMEM((NT, D, 128), F32), pltpu.VMEM((64, 128), U32),
            pltpu.VMEM((2, HD, BQ), U32),
            pltpu.VMEM((NB + 2, NT, 64, 128), U32), pltpu.VMEM((2, NT, 32, 128), U32),
            pltpu.VMEM((NB + 2, HD, BQ), U32),
            pltpu.VMEM((2, NT, BQ, 128), F32),
            pltpu.VMEM((2, NT, BQ + 16, 128), F32), pltpu.VMEM((2, NT, BQ + 16, 128), F32),
            pltpu.VMEM((NB + 2, BQ, 128), F32),
            pltpu.VMEM((2, D, BQ), F32), pltpu.VMEM((2, BQ, D), F32),
            pltpu.VMEM((64, D), U32), pltpu.VMEM((BQ, D), BF16),
            pltpu.VMEM((NB + 2, BQ, D), BF16),
            pltpu.SemaphoreType.DMA((9,)), pltpu.SemaphoreType.DMA((NS,)), pltpu.SemaphoreType.DMA(()),
        ],
        compiler_params=pltpu.CompilerParams(dimension_semantics=("arbitrary",),
                                             vmem_limit_bytes=100 * 1024 * 1024),
        name="gmix",
    )(A_x.reshape(S, D), A_wqkv, A_wo, B_wqkv, B_wo, gate_w)
    return out.reshape(1, S, D)
```
